```python
import os as _os
_os.environ.setdefault("JAX_PLATFORMS", "cpu")
import jax
import jax.numpy as jnp

def _softmax(x, axis=-1):
    return jax.nn.softmax(x, axis=axis)
def _gelu(x):
    return jax.nn.gelu(x, approximate=True)
def _silu(x):
    return jax.nn.silu(x)
def _sigmoid(x):
    return jax.nn.sigmoid(x)
def _layernorm(x, axis=-1, eps=1e-5):
    m = jnp.mean(x, axis=axis, keepdims=True)
    v = jnp.var(x, axis=axis, keepdims=True)
    return (x - m) / jnp.sqrt(v + eps)
def _scatter_add(tgt, idx, src, axis=0):
    return tgt.at[idx].add(src)
def _segment_sum(src, seg, n):
    return jax.ops.segment_sum(src, seg, n)
class _Rng:
    def __init__(self, key):
        self._k = key
    def _next(self):
        self._k, sub = jax.random.split(self._k)
        return sub
    def normal(self, shape):
        return jax.random.normal(self._next(), shape, dtype=jnp.bfloat16)
    def randint(self, lo, hi, shape):
        return jax.random.randint(self._next(), shape, lo, hi, dtype=jnp.int32)
    def uniform(self, shape, lo=0.0, hi=1.0):
        return jax.random.uniform(self._next(), shape, jnp.bfloat16, lo, hi)
    def permutation(self, n):
        return jax.random.permutation(self._next(), n)


kernel_name = 'parallel_sum__linear_kernel_hedgehog__dense_activation_gelu__prompt'

def setup_inputs():
    _rng = _Rng(jax.random.key(int.from_bytes(__import__("os").urandom(4), "little")))
    _w = (lambda a: (lambda t: t.astype(jnp.bfloat16) if jnp.issubdtype(t.dtype, jnp.floating) else t)(jnp.asarray(a)))
    def _A_setup():
        B, S, D, H = 1, 2048, 448, 16
        Dh = D // H
        return {
            "x": _w((lambda *s: _rng.normal(s) * 0.05)(B, S, D)),
            "wqkv": _w((lambda *s: _rng.normal(s) * 0.2)(D, 3 * D)),
            "w_phi": _w((lambda *s: _rng.normal(s) * 0.2)(H, Dh, Dh) * (Dh ** -0.5)),
            "wo": _w((lambda *s: _rng.normal(s) * 0.05)(D, D)),
        }
    _A_in = _A_setup()

    def _B_setup():
        B, S, D, F = 1, 2048, 448, 1792
        return {
            "x": _w((lambda *s: _rng.normal(s) * 0.05)(B, S, D)),
            "w1": _w((lambda *s: _rng.normal(s) * 0.2)(D, F) * (D ** -0.5)),
            "b1": _w((lambda *s: _rng.normal(s) * 0.2)(F) * 0.01),
            "w2": _w((lambda *s: _rng.normal(s) * 0.2)(F, D) * (F ** -0.5)),
            "b2": _w((lambda *s: _rng.normal(s) * 0.05)(D) * 0.01),
        }
    _B_in = _B_setup()

    return {
        "A_x": _A_in["x"],
        "A_wqkv": _A_in["wqkv"],
        "A_w_phi": _A_in["w_phi"],
        "A_wo": _A_in["wo"],
        "B_x": _B_in["x"],
        "B_w1": _B_in["w1"],
        "B_b1": _B_in["b1"],
        "B_w2": _B_in["w2"],
        "B_b2": _B_in["b2"],
    }

def reference(A_x, A_wqkv, A_w_phi, A_wo, B_x, B_w1, B_b1, B_w2, B_b2):
    def _A_ref(x, wqkv, w_phi, wo):
        B, S, D = x.shape
        H = 16; Dh = D // H
        qkv = (lambda x, *d: x.transpose(*d))((x @ wqkv).reshape(B, S, 3, H, Dh), 2, 0, 3, 1, 4)
        q, k, v = qkv[0], qkv[1], qkv[2]
        pq = jnp.einsum("bhsd,hdf->bhsf", q, w_phi)
        pk = jnp.einsum("bhsd,hdf->bhsf", k, w_phi)
        phi_q = jnp.concatenate([_softmax(pq, axis=-1), _softmax(-pq, axis=-1)], axis=-1)
        phi_k = jnp.concatenate([_softmax(pk, axis=-1), _softmax(-pk, axis=-1)], axis=-1)
        kv = jnp.einsum("bhsf,bhsd->bhfd", phi_k, v)
        z  = jnp.einsum("bhsf->bhf", phi_k)
        num = jnp.einsum("bhqf,bhfd->bhqd", phi_q, kv)
        den = jnp.einsum("bhqf,bhf->bhq", phi_q, z)[..., None] + 1e-6
        o = num / den
        return (lambda x, *d: x.transpose(*d))(o, 0, 2, 1, 3).reshape(B, S, D) @ wo

    def _B_ref(x, w1, b1, w2, b2):
        h = jnp.einsum("bsd,df->bsf", x, w1) + b1
        h = _gelu(h)
        return jnp.einsum("bsf,fd->bsd", h, w2) + b2

    x = A_x
    xn = _layernorm(x, axis=-1)
    return x + _A_ref(xn, A_wqkv, A_w_phi, A_wo) + _B_ref(xn, B_w1, B_b1, B_w2, B_b2)
```

```python
import jax
import jax.numpy as jnp
import jax.experimental.pallas as pl
import jax.experimental.pallas.tpu as pltpu

H = 16
HP = 32
G = 4
T = 512
NT = (((1,), (1,)), ((), ()))
TN = (((0,), (0,)), ((), ()))
f32 = jnp.float32
bf16 = jnp.bfloat16


def _dot(a, b, dims=None):
    if dims is None:
        return jnp.dot(a, b, preferred_element_type=f32)
    return jax.lax.dot_general(a, b, dims, preferred_element_type=f32)


def _iota(shape, d):
    return jax.lax.broadcasted_iota(jnp.int32, shape, d)


def _dual_exp(pT, dh):
    t = pT.shape[1]
    p = pT.reshape(H, HP, t)
    valid = _iota((H, HP, t), 1) < dh
    pp = jnp.where(valid, p, -jnp.inf)
    pn = jnp.where(valid, -p, -jnp.inf)
    ep = jnp.exp(pp - jnp.max(pp, axis=1, keepdims=True))
    en = jnp.exp(pn - jnp.max(pn, axis=1, keepdims=True))
    return ep, en


def _kernel(x_ref, wqkv_ref, wphi_ref, b1_ref, b2_ref, wo_hbm, w1_hbm, w2_hbm, o_ref,
            wqT, wkT, wv, xn_s, kv_s, m_s, zb_s, wo_s, w1_s, w2_s, sems, *, n, d, dh):
    i = pl.program_id(0)
    gd = G * dh
    copies = [pltpu.make_async_copy(wo_hbm, wo_s, sems.at[0]),
              pltpu.make_async_copy(w1_hbm, w1_s, sems.at[1]),
              pltpu.make_async_copy(w2_hbm, w2_s, sems.at[2])]

    @pl.when(i == 0)
    def _prep():
        for c in copies:
            c.start()
        wst = jnp.concatenate([wphi_ref[h].astype(f32) for h in range(H)], axis=0)
        e = (_iota((dh, H * HP), 0) == _iota((dh, H * HP), 1) % HP).astype(bf16)
        bd = _dot(wst.astype(bf16), e)
        bd = jnp.where(_iota((d, H * HP), 0) // dh == _iota((d, H * HP), 1) // HP, bd, 0.0).astype(bf16)
        wqT[...] = _dot(wqkv_ref[:, 0:d], bd).T.astype(bf16)
        wkT[...] = _dot(wqkv_ref[:, d:2 * d], bd).T.astype(bf16)
        zpad = jnp.zeros((d, 128 - gd), bf16)
        for g in range(H // G):
            wv[:, 128 * g:128 * (g + 1)] = jnp.concatenate(
                [wqkv_ref[:, 2 * d + gd * g:2 * d + gd * (g + 1)], zpad], axis=1)
        kv_s[...] = jnp.zeros_like(kv_s)

    @pl.when(i < n)
    def _phase1():
        x = x_ref[...].astype(f32)
        m = jnp.mean(x, axis=-1, keepdims=True)
        xc = x - m
        var = jnp.mean(xc * xc, axis=-1, keepdims=True)
        xn = (xc * jax.lax.rsqrt(var + 1e-5)).astype(bf16)
        xn_s[pl.ds(pl.multiple_of(i * T, T), T), :] = xn
        ep, en = _dual_exp(_dot(wkT[...], xn, NT), dh)
        fp = (ep / jnp.sum(ep, axis=1, keepdims=True)).astype(bf16)
        fn = (en / jnp.sum(en, axis=1, keepdims=True)).astype(bf16)
        v = _dot(xn, wv[...])
        v = jnp.where(_iota(v.shape, 1) % 128 == gd, 1.0, v).astype(bf16)
        for g in range(H // G):
            ph = jnp.concatenate([fp[G * g:G * (g + 1)].reshape(G * HP, T),
                                  fn[G * g:G * (g + 1)].reshape(G * HP, T)], axis=0)
            kv_s[g] += _dot(ph, v[:, 128 * g:128 * (g + 1)])

    @pl.when(i == n)
    def _mid():
        for c in copies:
            c.wait()
        for g in range(H // G):
            kv = kv_s[g]
            r = (_iota(kv.shape, 0) % (G * HP)) // HP
            c = _iota(kv.shape, 1)
            kvm = jnp.where(r == c // dh, kv, 0.0)[:, 0:gd].astype(bf16)
            mg = _dot(kvm, wo_s[gd * g:gd * (g + 1), :]).astype(bf16)
            m_s[G * HP * g:G * HP * (g + 1), :] = mg[0:G * HP]
            m_s[H * HP + G * HP * g:H * HP + G * HP * (g + 1), :] = mg[G * HP:]
            zb = jnp.broadcast_to(kv[:, gd:gd + 1], kv.shape)
            zb_s[G * HP * g:G * HP * (g + 1), :] = zb[0:G * HP]
            zb_s[H * HP + G * HP * g:H * HP + G * HP * (g + 1), :] = zb[G * HP:]

    @pl.when(i >= n)
    def _phase2():
        xn = xn_s[pl.ds(pl.multiple_of((i - n) * T, T), T), :]
        ep, en = _dual_exp(_dot(wqT[...], xn, NT), dh)
        zp = jnp.concatenate([zb_s[0:H * HP, :]] * (T // 128), axis=1).reshape(H, HP, T)
        zn = jnp.concatenate([zb_s[H * HP:, :]] * (T // 128), axis=1).reshape(H, HP, T)
        rp = 1.0 / jnp.sum(ep, axis=1, keepdims=True)
        rn = 1.0 / jnp.sum(en, axis=1, keepdims=True)
        den = (jnp.sum(ep * zp, axis=1, keepdims=True) * rp
               + jnp.sum(en * zn, axis=1, keepdims=True) * rn + 1e-6)
        rd = 1.0 / den
        fp = (ep * (rp * rd)).astype(bf16).reshape(H * HP, T)
        fn = (en * (rn * rd)).astype(bf16).reshape(H * HP, T)
        acc = _dot(jnp.concatenate([fp, fn], axis=0), m_s[...], TN)
        h = _dot(xn, w1_s[...]) + b1_ref[...].astype(f32)
        h = jax.nn.gelu(h, approximate=True).astype(bf16)
        acc = acc + _dot(h, w2_s[...])
        o_ref[...] = (x_ref[...].astype(f32) + acc + b2_ref[...].astype(f32)).astype(o_ref.dtype)


@jax.jit
def pallas_parallel_sum__linear_kernel_hedgehog__dense_activation_gelu__prompt_kernel(
    A_x, A_wqkv, A_w_phi, A_wo, B_x, B_w1, B_b1, B_w2, B_b2,
):
    del B_x
    b, s, d = A_x.shape
    f = B_w1.shape[1]
    dh = d // H
    n = b * s // T
    const = lambda shape: pl.BlockSpec(shape, lambda i: (0,) * len(shape))
    hbm = pl.BlockSpec(memory_space=pl.ANY)
    out = pl.pallas_call(
        lambda *r: _kernel(*r, n=n, d=d, dh=dh),
        grid=(2 * n,),
        in_specs=[
            pl.BlockSpec((T, d), lambda i: (i % n, 0)),
            const((d, 3 * d)), const((H, dh, dh)), const((1, f)), const((1, d)),
            hbm, hbm, hbm,
        ],
        out_specs=pl.BlockSpec((T, d), lambda i: (jnp.maximum(i - n, 0), 0)),
        out_shape=jax.ShapeDtypeStruct((b * s, d), A_x.dtype),
        scratch_shapes=[
            pltpu.VMEM((H * HP, d), bf16), pltpu.VMEM((H * HP, d), bf16),
            pltpu.VMEM((d, 128 * H // G), bf16), pltpu.VMEM((b * s, d), bf16),
            pltpu.VMEM((H // G, 2 * G * HP, 128), f32),
            pltpu.VMEM((2 * H * HP, d), bf16), pltpu.VMEM((2 * H * HP, 128), f32),
            pltpu.VMEM((d, d), bf16), pltpu.VMEM((d, f), bf16), pltpu.VMEM((f, d), bf16),
            pltpu.SemaphoreType.DMA((3,)),
        ],
        compiler_params=pltpu.CompilerParams(
            dimension_semantics=("arbitrary",), vmem_limit_bytes=100 * 1024 * 1024),
    )(A_x.reshape(b * s, d), A_wqkv, A_w_phi, B_b1.reshape(1, f), B_b2.reshape(1, d),
      A_wo, B_w1, B_w2)
    return out.reshape(b, s, d)
```

```python
import jax
import jax.numpy as jnp
import jax.experimental.pallas as pl
import jax.experimental.pallas.tpu as pltpu

H = 16
HP = 32
G = 4
T = 512
NT = (((1,), (1,)), ((), ()))
TN = (((0,), (0,)), ((), ()))
f32 = jnp.float32
bf16 = jnp.bfloat16


def _dot(a, b, dims=None):
    if dims is None:
        return jnp.dot(a, b, preferred_element_type=f32)
    return jax.lax.dot_general(a, b, dims, preferred_element_type=f32)


def _iota(shape, d):
    return jax.lax.broadcasted_iota(jnp.int32, shape, d)


def _dual_exp(pT, dh):
    t = pT.shape[1]
    p = pT.reshape(H, HP, t)
    valid = _iota((H, HP, t), 1) < dh
    pp = jnp.where(valid, p, -jnp.inf)
    pn = jnp.where(valid, -p, -jnp.inf)
    ep = jnp.exp(pp - jnp.max(pp, axis=1, keepdims=True))
    en = jnp.exp(pn - jnp.max(pn, axis=1, keepdims=True))
    return ep, en


def _kernel(x_ref, wqkv_ref, wphi_ref, b1_ref, b2_ref, wo_hbm, w1_hbm, w2_hbm, o_ref,
            wqT, wkT, wvT, xn_s, kv_s, mT_s, zb_s, wo_s, w1_s, w2T_s, w1T, b1_s, b2_s, sems, *, n, d, dh):
    i = pl.program_id(0)
    gd = G * dh
    copies = [pltpu.make_async_copy(wo_hbm, wo_s, sems.at[0]),
              pltpu.make_async_copy(w1_hbm, w1_s, sems.at[1]),
              pltpu.make_async_copy(w2_hbm, w2T_s, sems.at[2])]

    @pl.when(i == 0)
    def _prep():
        for c in copies:
            c.start()
        wst = jnp.concatenate([wphi_ref[h].astype(f32) for h in range(H)], axis=0)
        e = (_iota((dh, H * HP), 0) == _iota((dh, H * HP), 1) % HP).astype(bf16)
        bd = _dot(wst.astype(bf16), e)
        bd = jnp.where(_iota((d, H * HP), 0) // dh == _iota((d, H * HP), 1) // HP, bd, 0.0).astype(bf16)
        wqT[...] = _dot(wqkv_ref[:, 0:d], bd).T.astype(bf16)
        wkT[...] = _dot(wqkv_ref[:, d:2 * d], bd).T.astype(bf16)
        zpad = jnp.zeros((d, 128 - gd), bf16)
        for g in range(H // G):
            wvT[128 * g:128 * (g + 1), :] = jnp.concatenate(
                [wqkv_ref[:, 2 * d + gd * g:2 * d + gd * (g + 1)], zpad], axis=1).T
        b1_s[...] = jnp.broadcast_to(b1_ref[...].astype(f32), (128, b1_s.shape[0])).T
        b2_s[...] = jnp.broadcast_to(b2_ref[...].astype(f32), (128, d)).T
        kv_s[...] = jnp.zeros_like(kv_s)

    @pl.when(i < n)
    def _phase1():
        x = x_ref[...].astype(f32)
        m = jnp.mean(x, axis=0, keepdims=True)
        xc = x - m
        var = jnp.mean(xc * xc, axis=0, keepdims=True)
        xn = (xc * jax.lax.rsqrt(var + 1e-5)).astype(bf16)
        xn_s[i] = xn
        ep, en = _dual_exp(_dot(wkT[...], xn), dh)
        fp = (ep / jnp.sum(ep, axis=1, keepdims=True)).astype(bf16)
        fn = (en / jnp.sum(en, axis=1, keepdims=True)).astype(bf16)
        v = _dot(wvT[...], xn)
        v = jnp.where(_iota(v.shape, 0) % 128 == gd, 1.0, v).astype(bf16)
        for g in range(H // G):
            ph = jnp.concatenate([fp[G * g:G * (g + 1)].reshape(G * HP, T),
                                  fn[G * g:G * (g + 1)].reshape(G * HP, T)], axis=0)
            kv_s[g] += _dot(ph, v[128 * g:128 * (g + 1), :], NT)

    @pl.when(i == n)
    def _mid():
        for c in copies:
            c.wait()
        w1T[...] = w1_s[...].T
        for g in range(H // G):
            kv = kv_s[g]
            r = (_iota(kv.shape, 0) % (G * HP)) // HP
            c = _iota(kv.shape, 1)
            kvm = jnp.where(r == c // dh, kv, 0.0)[:, 0:gd].astype(bf16)
            mg = _dot(kvm, wo_s[gd * g:gd * (g + 1), :]).astype(bf16)
            mT_s[:, G * HP * g:G * HP * (g + 1)] = mg[0:G * HP].T
            mT_s[:, H * HP + G * HP * g:H * HP + G * HP * (g + 1)] = mg[G * HP:].T
            zb = jnp.broadcast_to(kv[:, gd:gd + 1], kv.shape)
            zb_s[G * HP * g:G * HP * (g + 1), :] = zb[0:G * HP]
            zb_s[H * HP + G * HP * g:H * HP + G * HP * (g + 1), :] = zb[G * HP:]

    @pl.when(i >= n)
    def _phase2():
        xn = xn_s[i - n]
        ep, en = _dual_exp(_dot(wqT[...], xn), dh)
        zp = jnp.concatenate([zb_s[0:H * HP, :]] * (T // 128), axis=1).reshape(H, HP, T)
        zn = jnp.concatenate([zb_s[H * HP:, :]] * (T // 128), axis=1).reshape(H, HP, T)
        rp = 1.0 / jnp.sum(ep, axis=1, keepdims=True)
        rn = 1.0 / jnp.sum(en, axis=1, keepdims=True)
        den = (jnp.sum(ep * zp, axis=1, keepdims=True) * rp
               + jnp.sum(en * zn, axis=1, keepdims=True) * rn + 1e-6)
        rd = 1.0 / den
        fp = (ep * (rp * rd)).astype(bf16).reshape(H * HP, T)
        fn = (en * (rn * rd)).astype(bf16).reshape(H * HP, T)
        acc = _dot(mT_s[...], jnp.concatenate([fp, fn], axis=0))
        h = _dot(w1T[...], xn) + jnp.concatenate([b1_s[...]] * (T // 128), axis=1)
        h = jax.nn.gelu(h, approximate=True).astype(bf16)
        acc = acc + _dot(w2T_s[...], h)
        o_ref[...] = (x_ref[...].astype(f32) + acc
                      + jnp.concatenate([b2_s[...]] * (T // 128), axis=1)).astype(o_ref.dtype)


@jax.jit
def pallas_parallel_sum__linear_kernel_hedgehog__dense_activation_gelu__prompt_kernel(
    A_x, A_wqkv, A_w_phi, A_wo, B_x, B_w1, B_b1, B_w2, B_b2,
):
    del B_x
    b, s, d = A_x.shape
    f = B_w1.shape[1]
    dh = d // H
    n = b * s // T
    const = lambda shape: pl.BlockSpec(shape, lambda i: (0,) * len(shape))
    hbm = pl.BlockSpec(memory_space=pl.ANY)
    out = pl.pallas_call(
        lambda *r: _kernel(*r, n=n, d=d, dh=dh),
        grid=(2 * n,),
        in_specs=[
            pl.BlockSpec((d, T), lambda i: (0, i % n)),
            const((d, 3 * d)), const((H, dh, dh)), const((1, f)), const((1, d)),
            hbm, hbm, hbm,
        ],
        out_specs=pl.BlockSpec((d, T), lambda i: (0, jnp.maximum(i - n, 0))),
        out_shape=jax.ShapeDtypeStruct((d, b * s), A_x.dtype),
        scratch_shapes=[
            pltpu.VMEM((H * HP, d), bf16), pltpu.VMEM((H * HP, d), bf16),
            pltpu.VMEM((128 * H // G, d), bf16), pltpu.VMEM((n, d, T), bf16),
            pltpu.VMEM((H // G, 2 * G * HP, 128), f32),
            pltpu.VMEM((d, 2 * H * HP), bf16), pltpu.VMEM((2 * H * HP, 128), f32),
            pltpu.VMEM((d, d), bf16), pltpu.VMEM((d, f), bf16), pltpu.VMEM((d, f), bf16),
            pltpu.VMEM((f, d), bf16), pltpu.VMEM((f, 128), f32), pltpu.VMEM((d, 128), f32),
            pltpu.SemaphoreType.DMA((3,)),
        ],
        compiler_params=pltpu.CompilerParams(
            dimension_semantics=("arbitrary",), vmem_limit_bytes=100 * 1024 * 1024),
    )(A_x.reshape(b * s, d).T, A_wqkv, A_w_phi, B_b1.reshape(1, f), B_b2.reshape(1, d),
      A_wo, B_w1, B_w2.T)
    return out.T.reshape(b, s, d)
```

```python
import jax
import jax.numpy as jnp
import jax.experimental.pallas as pl
import jax.experimental.pallas.tpu as pltpu

H = 16
G = 8
NG = H // G
VP = 16
T = 512
NT = (((1,), (1,)), ((), ()))
TN = (((0,), (0,)), ((), ()))
f32 = jnp.float32
bf16 = jnp.bfloat16


def _dot(a, b, dims=None):
    if dims is None:
        return jnp.dot(a, b, preferred_element_type=f32)
    return jax.lax.dot_general(a, b, dims, preferred_element_type=f32)


def _iota(shape, d):
    return jax.lax.broadcasted_iota(jnp.int32, shape, d)


def _dual_exp(pT, dh):
    p = pT.reshape(NG, dh, G, pT.shape[1])
    ep = jnp.exp(p - jnp.max(p, axis=1, keepdims=True))
    en = jnp.exp(jnp.min(p, axis=1, keepdims=True) - p)
    return ep, en


def _kernel(x_ref, wqkv_ref, wphi_ref, b1_ref, b2_ref, wo_hbm, w1_hbm, w2_hbm, o_ref,
            wqT, wkT, wvT, xn_s, kv_s, mT_all, zb_s, wo_s, w1_s, w2T_s, w1T, b1_s, b2_s, bd_s, sems, *, n, d, dh):
    i = pl.program_id(0)
    gd = G * dh
    vg = gd + VP
    copies = [pltpu.make_async_copy(wo_hbm, wo_s, sems.at[0]),
              pltpu.make_async_copy(w1_hbm, w1_s, sems.at[1]),
              pltpu.make_async_copy(w2_hbm, w2T_s, sems.at[2])]

    @pl.when(i == 0)
    def _prep():
        for c in copies:
            c.start()
        wp = wphi_ref[...].astype(f32)
        wst = jnp.concatenate([wp[:, h, :] for h in range(H)], axis=0)
        e = (_iota((dh, gd), 0) == _iota((dh, gd), 1) // G).astype(bf16)
        bd = _dot(wst.astype(bf16), e)
        bd = jnp.where((_iota((d, gd), 0) % gd) // dh == _iota((d, gd), 1) % G, bd, 0.0).astype(bf16)
        bd_s[...] = bd
        wvt = wqkv_ref[:, 2 * d:3 * d].T
        for g in range(NG):
            bg = bd[gd * g:gd * (g + 1)]
            wkT[gd * g:gd * (g + 1), :] = _dot(wqkv_ref[:, d + gd * g:d + gd * (g + 1)], bg).T.astype(bf16)
            wvT[vg * g:vg * g + gd, :] = wvt[gd * g:gd * (g + 1)]
            wvT[vg * g + gd:vg * (g + 1), :] = jnp.zeros((VP, d), bf16)
        kv_s[...] = jnp.zeros_like(kv_s)

    def _phase1(extra):
        extra()
        x = x_ref[...].astype(f32)
        m = jnp.mean(x, axis=0, keepdims=True)
        xc = x - m
        var = jnp.mean(xc * xc, axis=0, keepdims=True)
        xn = (xc * jax.lax.rsqrt(var + 1e-5)).astype(bf16)
        xn_s[i] = xn
        ep, en = _dual_exp(_dot(wkT[...], xn), dh)
        fp = ep * (1.0 / jnp.sum(ep, axis=1, keepdims=True))
        fn = en * (1.0 / jnp.sum(en, axis=1, keepdims=True))
        v = _dot(wvT[...], xn)
        v = jnp.where(_iota(v.shape, 0) % vg == gd, 1.0, v).astype(bf16)
        for g in range(NG):
            ph = jnp.concatenate([fp[g].reshape(gd, T), fn[g].reshape(gd, T)], axis=0).astype(bf16)
            kv_s[g] += _dot(ph, v[vg * g:vg * (g + 1), :], NT)

    def _late_prep():
        w1T[...] = w1_s[...].T
        for g in range(NG):
            bg = bd_s[gd * g:gd * (g + 1), :]
            wqT[gd * g:gd * (g + 1), :] = _dot(wqkv_ref[:, gd * g:gd * (g + 1)], bg).T.astype(bf16)
        b1_s[...] = jnp.broadcast_to(b1_ref[...].astype(f32).reshape(1, -1), (128, b1_s.shape[0])).T
        b2_s[...] = jnp.broadcast_to(b2_ref[...].astype(f32).reshape(1, -1), (128, d)).T

    @pl.when(i == n - 1)
    def _():
        copies[1].wait()
        _phase1(_late_prep)

    @pl.when(i < n - 1)
    def _():
        _phase1(lambda: None)

    @pl.when(i == n)
    def _mid():
        for c in copies[::2]:
            c.wait()
        for g in range(NG):
            kv = kv_s[g]
            kvm = jnp.where(_iota(kv.shape, 0) % G == _iota(kv.shape, 1) // dh, kv, 0.0)
            mg = _dot(kvm[:, 0:gd].astype(bf16), wo_s[gd * g:gd * (g + 1), :])
            mT_all[:, 2 * gd * g:2 * gd * (g + 1)] = mg.T.astype(bf16)
            zb_s[g] = jnp.broadcast_to(kv[:, gd:gd + 1], (2 * gd, 128))

    @pl.when(i >= n)
    def _phase2():
        xn = xn_s[i - n]
        ep, en = _dual_exp(_dot(wqT[...], xn), dh)
        zp = jnp.concatenate([zb_s[:, 0:gd, :]] * (T // 128), axis=2).reshape(NG, dh, G, T)
        zn = jnp.concatenate([zb_s[:, gd:, :]] * (T // 128), axis=2).reshape(NG, dh, G, T)
        rp = 1.0 / jnp.sum(ep, axis=1, keepdims=True)
        rn = 1.0 / jnp.sum(en, axis=1, keepdims=True)
        den = (jnp.sum(ep * zp, axis=1, keepdims=True) * rp
               + jnp.sum(en * zn, axis=1, keepdims=True) * rn + 1e-6)
        rd = 1.0 / den
        fp = ep * (rp * rd)
        fn = en * (rn * rd)
        ph = jnp.concatenate([x[g].reshape(gd, T) for g in range(NG) for x in (fp, fn)], axis=0)
        acc = _dot(mT_all[...], ph.astype(bf16))
        h = _dot(w1T[...], xn) + jnp.concatenate([b1_s[...]] * (T // 128), axis=1)
        h = jax.nn.gelu(h, approximate=True).astype(bf16)
        acc = acc + _dot(w2T_s[...], h)
        o_ref[...] = (x_ref[...].astype(f32) + acc
                      + jnp.concatenate([b2_s[...]] * (T // 128), axis=1)).astype(o_ref.dtype)


@jax.jit
def pallas_parallel_sum__linear_kernel_hedgehog__dense_activation_gelu__prompt_kernel(
    A_x, A_wqkv, A_w_phi, A_wo, B_x, B_w1, B_b1, B_w2, B_b2,
):
    del B_x
    b, s, d = A_x.shape
    f = B_w1.shape[1]
    dh = d // H
    n = b * s // T
    const = lambda shape: pl.BlockSpec(shape, lambda i: (0,) * len(shape))
    hbm = pl.BlockSpec(memory_space=pl.ANY)
    out = pl.pallas_call(
        lambda *r: _kernel(*r, n=n, d=d, dh=dh),
        grid=(2 * n,),
        in_specs=[
            pl.BlockSpec((d, T), lambda i: (0, i % n)),
            const((d, 3 * d)), const((dh, H, dh)), const((f,)), const((d,)),
            hbm, hbm, hbm,
        ],
        out_specs=pl.BlockSpec((d, T), lambda i: (0, jnp.maximum(i - n, 0))),
        out_shape=jax.ShapeDtypeStruct((d, b * s), A_x.dtype),
        scratch_shapes=[
            pltpu.VMEM((d, d), bf16), pltpu.VMEM((d, d), bf16),
            pltpu.VMEM((NG * (G * dh + VP), d), bf16), pltpu.VMEM((n, d, T), bf16),
            pltpu.VMEM((NG, 2 * G * dh, G * dh + VP), f32),
            pltpu.VMEM((d, 2 * d), bf16), pltpu.VMEM((NG, 2 * G * dh, 128), f32),
            pltpu.VMEM((d, d), bf16), pltpu.VMEM((d, f), bf16), pltpu.VMEM((d, f), bf16),
            pltpu.VMEM((f, d), bf16), pltpu.VMEM((f, 128), f32), pltpu.VMEM((d, 128), f32),
            pltpu.VMEM((d, G * dh), bf16),
            pltpu.SemaphoreType.DMA((3,)),
        ],
        compiler_params=pltpu.CompilerParams(
            dimension_semantics=("arbitrary",), vmem_limit_bytes=100 * 1024 * 1024),
    )(A_x.reshape(b * s, d).T, A_wqkv, A_w_phi.transpose(1, 0, 2), B_b1, B_b2,
      A_wo, B_w1, B_w2.T)
    return out.T.reshape(b, s, d)
```
